```python
import os as _os
_os.environ.setdefault("JAX_PLATFORMS", "cpu")
import jax
import jax.numpy as jnp

def _softmax(x, axis=-1):
    return jax.nn.softmax(x, axis=axis)
def _gelu(x):
    return jax.nn.gelu(x, approximate=True)
def _silu(x):
    return jax.nn.silu(x)
def _sigmoid(x):
    return jax.nn.sigmoid(x)
def _layernorm(x, axis=-1, eps=1e-5):
    m = jnp.mean(x, axis=axis, keepdims=True)
    v = jnp.var(x, axis=axis, keepdims=True)
    return (x - m) / jnp.sqrt(v + eps)
def _scatter_add(tgt, idx, src, axis=0):
    return tgt.at[idx].add(src)
def _segment_sum(src, seg, n):
    return jax.ops.segment_sum(src, seg, n)
class _Rng:
    def __init__(self, key):
        self._k = key
    def _next(self):
        self._k, sub = jax.random.split(self._k)
        return sub
    def normal(self, shape):
        return jax.random.normal(self._next(), shape, dtype=jnp.bfloat16)
    def randint(self, lo, hi, shape):
        return jax.random.randint(self._next(), shape, lo, hi, dtype=jnp.int32)
    def uniform(self, shape, lo=0.0, hi=1.0):
        return jax.random.uniform(self._next(), shape, jnp.bfloat16, lo, hi)
    def permutation(self, n):
        return jax.random.permutation(self._next(), n)


kernel_name = 'sequential_preLN__sliding_local_dilated__dense_activation_mish__prompt'

def setup_inputs():
    _rng = _Rng(jax.random.key(int.from_bytes(__import__("os").urandom(4), "little")))
    _w = (lambda a: (lambda t: t.astype(jnp.bfloat16) if jnp.issubdtype(t.dtype, jnp.floating) else t)(jnp.asarray(a)))
    def _A_setup():
        B, S, D = 1, 2048, 512
        return {
            "x": _w((lambda *s: _rng.normal(s) * 0.05)(B, S, D)),
            "wqkv": _w((lambda *s: _rng.normal(s) * 0.05)(D, 3 * D)),
            "wo": _w((lambda *s: _rng.normal(s) * 0.05)(D, D)),
        }
    _A_in = _A_setup()

    def _B_setup():
        B, S, D, F = 1, 2048, 512, 1376
        return {
            "x": _w((lambda *s: _rng.normal(s) * 0.05)(B, S, D)),
            "w1": _w((lambda *s: _rng.normal(s) * 1.6)(D, F) * (D ** -0.5)),
            "b1": _w((lambda *s: _rng.normal(s) * 0.1)(F)),
            "w2": _w((lambda *s: _rng.normal(s) * 0.1)(F, D) * (F ** -0.5)),
        }
    _B_in = _B_setup()

    return {
        "A_x": _A_in["x"],
        "A_wqkv": _A_in["wqkv"],
        "A_wo": _A_in["wo"],
        "B_x": _B_in["x"],
        "B_w1": _B_in["w1"],
        "B_b1": _B_in["b1"],
        "B_w2": _B_in["w2"],
    }

def reference(A_x, A_wqkv, A_wo, B_x, B_w1, B_b1, B_w2):
    def _A_ref(x, wqkv, wo):
        B, S, D = x.shape
        H = 32; Dh = D // H
        W, dil = 8, 2
        qkv = (lambda x, *d: x.transpose(*d))((x @ wqkv).reshape(B, S, 3, H, Dh), 2, 0, 3, 1, 4)
        q, k, v = qkv[0], qkv[1], qkv[2]
        scale = Dh ** -0.5
        pos = jnp.arange(S)
        off = jnp.arange(W) * dil
        idx = pos[:, None] - off[None, :]
        mask = idx >= 0
        idx_c = jnp.where(mask, idx, 0).reshape(-1)
        kg = k[:, :, idx_c, :].reshape(B, H, S, W, Dh)
        vg = v[:, :, idx_c, :].reshape(B, H, S, W, Dh)
        logits = jnp.einsum("bhsd,bhswd->bhsw", q, kg) * scale
        logits = jnp.where(mask[None, None, :, :], logits, -1e9)
        attn = _softmax(logits, axis=-1)
        o = jnp.einsum("bhsw,bhswd->bhsd", attn, vg)
        return (lambda x, *d: x.transpose(*d))(o, 0, 2, 1, 3).reshape(B, S, D) @ wo

    def _B_ref(x, w1, b1, w2):
        h = jnp.einsum("bsd,df->bsf", x, w1) + b1
        sp = jnp.log1p(jnp.exp(-jnp.abs(h))) + jnp.where(h > 0, h, jnp.zeros_like(h))
        act = h * jnp.tanh(sp)
        return jnp.einsum("bsf,fd->bsd", act, w2)

    x = A_x
    h = x + _A_ref(_layernorm(x, axis=-1), A_wqkv, A_wo)
    h2 = h + _B_ref(_layernorm(h, axis=-1), B_w1, B_b1, B_w2)
    return h2
```

```python
import jax
import jax.numpy as jnp
from jax.experimental import pallas as pl
from jax.experimental.pallas import tpu as pltpu

S, D, F = 2048, 512, 1376
H, DH, W, DIL = 32, 16, 8, 2
FP = 1408
T = 128
NB = S // T
H2 = T // 2
CH = 16
LNCH = 32
HALO = 16
OSPLIT = 2
LOG2E = 1.4426950408889634
NT = (((1,), (1,)), ((), ()))
bf16, f32, u32 = jnp.bfloat16, jnp.float32, jnp.uint32


def _schedule():
    late = ",".join(f"x{i}" for i in range(8, NB))
    s = f"S[x0,x1,wq,wk,x2,x3,wv,wo,x4,x5,b1,w1,x6,x7,w2,{late}] "
    s += "B[x0,x1,wq] Mq Q0 Q1 B[wk,x2,x3] Pk Q2 Q3 K0 K1 K2 "
    s += "B[wv,wo,x4,x5] Pv K3 V0 V1 V2 V3 Po K4 K5 V4 V5 WO0 WO1 WO2 WO3 Q4 Q5 L2_0 L2_1 L2_2 L2_3 "
    s += f"B[b1,w1,x6,x7] Fb W1_0 W1_1 B[w2,{late}] W2_0 W1_2 Q6 K6 V6 W1_3 W2_1 W2_2 "
    for i in range(5, NB):
        s += f"WO{i - 1} "
        if i + 2 < NB:
            s += f"V{i + 2} Q{i + 2} K{i + 2} "
        s += f"W2_{i - 2} W1_{i - 1} "
    s += f"WO{NB - 1} W2_{NB - 2} W1_{NB - 1} W2_{NB - 1}"
    return s.split()


def _layernorm(x):
    m = jnp.mean(x, axis=-1, keepdims=True)
    xc = x - m
    v = jnp.mean(xc * xc, axis=-1, keepdims=True)
    return xc * jax.lax.rsqrt(v + 1e-5)


def _mish(h):
    e = jnp.exp2(jnp.minimum(h * LOG2E, 60.0))
    n = e * (e + 2.0)
    return h * (n * pltpu.reciprocal(n + 2.0, approx=True))


def _as_bf16(x):
    return pltpu.bitcast(x, bf16)


def _as_u32(x):
    return pltpu.bitcast(x, u32)


def _kernel(x_hbm, wqkv_hbm, wo_hbm, w1t_hbm, b1_hbm, w2_hbm, o_hbm,
            x_buf, o_buf, wraw, wtmp, woraw, wqkvT, wo_p, w1t, b1v, b1f, w2,
            xn_scr, q_scr, k_scr, v_scr, a_scr, h_scr, hn_scr, act_scr, sems, osem):
    def in_copies(name):
        if name[0] == "x":
            i = int(name[1:])
            return [pltpu.make_async_copy(x_hbm.at[0, pl.ds(i * T, T), :], x_buf.at[pl.ds(i * T, T), :], sems.at[i])]
        if name in ("wq", "wk", "wv"):
            p = "qkv".index(name[1])
            return [pltpu.make_async_copy(wqkv_hbm.at[:, pl.ds(p * D, D)], wraw.at[p].bitcast(bf16), sems.at[NB + p])]
        if name == "wo":
            return [pltpu.make_async_copy(wo_hbm.at[:, pl.ds(j * 128, 128)], woraw.at[j].bitcast(bf16), sems.at[NB + 3])
                    for j in range(4)]
        if name == "w1":
            return [pltpu.make_async_copy(w1t_hbm, w1t.at[pl.ds(0, F // 2)].bitcast(bf16), sems.at[NB + 4])]
        if name == "w2":
            return [pltpu.make_async_copy(w2_hbm, w2.at[pl.ds(0, F // 2)].bitcast(bf16), sems.at[NB + 5])]
        assert name == "b1"
        return [pltpu.make_async_copy(b1_hbm, b1v, sems.at[NB + 6])]

    def out_copies(i):
        rows = pl.ds(i * T, T)
        if i >= NB - OSPLIT:
            return [pltpu.make_async_copy(o_buf.at[rows, pl.ds(c * 128, 128)], o_hbm.at[0, rows, pl.ds(c * 128, 128)],
                                          osem.at[i]) for c in range(4)]
        return [pltpu.make_async_copy(o_buf.at[rows, :], o_hbm.at[0, rows, :], osem.at[i])]

    def unpack(w):
        lo = pltpu.bitcast(w << 16, f32)
        hi = pltpu.bitcast(w & jnp.uint32(0xFFFF0000), f32)
        return lo.astype(bf16), hi.astype(bf16)

    def prep_w_xlu(p):
        for j in range(4):
            wtmp[p, j] = _as_u32(_as_bf16(wraw[p, pl.ds(j * 64, 64), :]).T)
        for j in range(4):
            for dp in range(DH // 2):
                lo, hi = unpack(wtmp[p, j, pl.ds(dp, H, stride=DH // 2), :])
                wqkvT[pl.ds(p * (D // 2) + (2 * dp) * (H // 2), H // 2), j * 128:(j + 1) * 128] = _as_u32(lo)
                wqkvT[pl.ds(p * (D // 2) + (2 * dp + 1) * (H // 2), H // 2), j * 128:(j + 1) * 128] = _as_u32(hi)

    def prep_w_mxu(p):
        mi = jax.lax.broadcasted_iota(jnp.int32, (128, 128), 0)
        ni = jax.lax.broadcasted_iota(jnp.int32, (128, 128), 1)
        sel = jnp.where(ni == (mi % 8) * DH + mi // 8, 1.0, 0.0).astype(bf16)
        for a in range(2):
            outs = [jax.lax.dot_general(sel, _as_bf16(wraw[p, :, i * 128:(i + 1) * 128]), NT, preferred_element_type=f32)
                    for i in (2 * a, 2 * a + 1)]
            for d in range(DH):
                blk = jnp.concatenate([outs[0][d * 8:(d + 1) * 8], outs[1][d * 8:(d + 1) * 8]], axis=0)
                wqkvT[pl.ds((p * D + d * H + 16 * a) // 2, 8), :] = _as_u32(blk.astype(bf16))

    def prep_wo():
        for j in range(4):
            for dp in range(DH // 2):
                lo, hi = unpack(woraw[j, pl.ds(dp, H, stride=DH // 2), :])
                wo_p[pl.ds((2 * dp) * (H // 2), H // 2), j * 128:(j + 1) * 128] = _as_u32(lo)
                wo_p[pl.ds((2 * dp + 1) * (H // 2), H // 2), j * 128:(j + 1) * 128] = _as_u32(hi)

    def ln1(i):
        for r in range(i * T, (i + 1) * T, LNCH):
            xn_scr[pl.ds(r // 2, LNCH // 2), :] = _as_u32(_layernorm(x_buf[pl.ds(r, LNCH), :].astype(f32)).astype(bf16))

    def proj(i, p):
        dst, off = ((q_scr, 0), (k_scr, HALO), (v_scr, HALO))[p]
        for c in range(4):
            xn = _as_bf16(xn_scr[pl.ds(i * H2, H2), :])
            w = _as_bf16(wqkvT[pl.ds((p * D + c * 128) // 2, 64), :])
            dst[c, pl.ds(off + i * T, T), :] = jax.lax.dot_general(xn, w, NT, preferred_element_type=f32)

    def attention(i):
        for r in range(i * T, (i + 1) * T, CH):
            q = [q_scr[c, pl.ds(r, CH), :] for c in range(4)]
            part = []
            for w in range(W):
                acc = None
                for c in range(4):
                    p = q[c] * k_scr[c, pl.ds(HALO + r - DIL * w, CH), :]
                    acc = p if acc is None else acc + p
                part.append(acc)
            part = [p + pltpu.roll(p, 64, 1) for p in part]
            logits = [p + pltpu.roll(p, 32, 1) for p in part]
            for w in range(W):
                if r < DIL * w:
                    pos = jax.lax.broadcasted_iota(jnp.int32, (CH, 128), 0) + (r - DIL * w)
                    logits[w] = jnp.where(pos >= 0, logits[w], -1e30)
            m = logits[0]
            for w in range(1, W):
                m = jnp.maximum(m, logits[w])
            e = [jnp.exp2((logits[w] - m) * (DH ** -0.5 * LOG2E)) for w in range(W)]
            s = e[0]
            for w in range(1, W):
                s = s + e[w]
            rs = pltpu.reciprocal(s, approx=True)
            for c in range(4):
                acc = None
                for w in range(W):
                    p = e[w] * v_scr[c, pl.ds(HALO + r - DIL * w, CH), :]
                    acc = p if acc is None else acc + p
                a_scr[pl.ds(r // 2, CH // 2), c * 128:(c + 1) * 128] = _as_u32((acc * rs).astype(bf16))

    def out_proj(i):
        for c in range(4):
            a = _as_bf16(a_scr[pl.ds(i * H2, H2), :])
            x = x_buf[pl.ds(i * T, T), c * 128:(c + 1) * 128].astype(f32)
            h_scr[pl.ds(i * T, T), c * 128:(c + 1) * 128] = x + jnp.dot(
                a, _as_bf16(wo_p[:, c * 128:(c + 1) * 128]), preferred_element_type=f32)

    def ln2(i):
        for r in range(i * T, (i + 1) * T, LNCH):
            hn_scr[pl.ds(r // 2, LNCH // 2), :] = _as_u32(_layernorm(h_scr[pl.ds(r, LNCH), :]).astype(bf16))

    def ffn1(i):
        for j in range(FP // 128):
            hn = _as_bf16(hn_scr[pl.ds(i * H2, H2), :])
            hh = jax.lax.dot_general(hn, _as_bf16(w1t[pl.ds(j * 64, 64), :]), NT, preferred_element_type=f32)
            hh = hh + b1f[:, j * 128:(j + 1) * 128]
            act_scr[pl.ds(i * H2, H2), j * 128:(j + 1) * 128] = _as_u32(_mish(hh).astype(bf16))

    def ffn2(i):
        cps = out_copies(i)
        for c in range(4):
            act = _as_bf16(act_scr[pl.ds(i * H2, H2), :])
            y = jnp.dot(act, _as_bf16(w2[:, c * 128:(c + 1) * 128]), preferred_element_type=f32)
            o_buf[pl.ds(i * T, T), c * 128:(c + 1) * 128] = (h_scr[pl.ds(i * T, T), c * 128:(c + 1) * 128] + y).astype(bf16)
            if len(cps) == 4:
                cps[c].start()
        if len(cps) == 1:
            cps[0].start()

    done = set()

    def once(name, fn, i):
        if (name, i) not in done:
            done.add((name, i))
            fn(i)

    for tok in _schedule():
        if tok[0] in "SB" and tok[1] == "[":
            for name in tok[2:-1].split(","):
                for cp in in_copies(name):
                    cp.start() if tok[0] == "S" else cp.wait()
            if tok[0] == "S":
                zero = jnp.zeros((HALO, 128), f32)
                for c in range(4):
                    k_scr[c, pl.ds(0, HALO), :] = zero
                    v_scr[c, pl.ds(0, HALO), :] = zero
                zpad = jnp.zeros(((FP - F) // 2, D), u32)
                w1t[pl.ds(F // 2, (FP - F) // 2), :] = zpad
                w2[pl.ds(F // 2, (FP - F) // 2), :] = zpad
                b1f[...] = jnp.zeros((1, FP), f32)
        elif tok == "Fb":
            b1f[:, pl.ds(0, F)] = b1v[...].astype(f32).reshape(1, F)
        elif tok == "Po":
            prep_wo()
        elif tok[0] == "P":
            prep_w_xlu("qkv".index(tok[1]))
        elif tok[0] == "M":
            prep_w_mxu("qkv".index(tok[1]))
        elif tok[0] in "QKV":
            i = int(tok[1:])
            once("ln1", ln1, i)
            proj(i, "QKV".index(tok[0]))
            done.add((tok[0], i))
        elif tok[:2] == "WO":
            i = int(tok[2:])
            assert all((n, j) in done for n in "KV" for j in range(max(i - 1, 0), i + 1)) and ("Q", i) in done
            once("att", attention, i)
            out_proj(i)
            done.add(("WO", i))
        elif tok[:3] == "L2_":
            once("ln2", ln2, int(tok[3:]))
        elif tok[:3] == "W1_":
            i = int(tok[3:])
            assert ("WO", i) in done
            once("ln2", ln2, i)
            ffn1(i)
            done.add(("W1", i))
        else:
            assert tok[:3] == "W2_"
            i = int(tok[3:])
            assert ("W1", i) in done
            ffn2(i)
            done.add(("W2", i))
    for i in range(NB):
        assert ("W2", i) in done
        for cp in out_copies(i):
            cp.wait()


@jax.jit
def pallas_sequential_preLN__sliding_local_dilated__dense_activation_mish__prompt_kernel(
    A_x: jax.Array,
    A_wqkv: jax.Array,
    A_wo: jax.Array,
    B_x: jax.Array,
    B_w1: jax.Array,
    B_b1: jax.Array,
    B_w2: jax.Array,
):
    del B_x
    assert A_x.shape == (1, S, D) and B_w1.shape == (D, F)
    hbm = pl.BlockSpec(memory_space=pltpu.HBM)
    return pl.pallas_call(
        _kernel,
        in_specs=[hbm] * 6,
        out_specs=hbm,
        out_shape=jax.ShapeDtypeStruct((1, S, D), A_x.dtype),
        scratch_shapes=[
            pltpu.VMEM((S, D), bf16),
            pltpu.VMEM((S, D), bf16),
            pltpu.VMEM((3, D // 2, D), u32),
            pltpu.VMEM((3, 4, D // 2, 128), u32),
            pltpu.VMEM((4, D // 2, 128), u32),
            pltpu.VMEM((3 * D // 2, D), u32),
            pltpu.VMEM((D // 2, D), u32),
            pltpu.VMEM((FP // 2, D), u32),
            pltpu.VMEM((F,), bf16),
            pltpu.VMEM((1, FP), f32),
            pltpu.VMEM((FP // 2, D), u32),
            pltpu.VMEM((S // 2, D), u32),
            pltpu.VMEM((4, S, 128), f32),
            pltpu.VMEM((4, S + HALO, 128), f32),
            pltpu.VMEM((4, S + HALO, 128), f32),
            pltpu.VMEM((S // 2, D), u32),
            pltpu.VMEM((S, D), f32),
            pltpu.VMEM((S // 2, D), u32),
            pltpu.VMEM((S // 2, FP), u32),
            pltpu.SemaphoreType.DMA((NB + 7,)),
            pltpu.SemaphoreType.DMA((NB,)),
        ],
        compiler_params=pltpu.CompilerParams(vmem_limit_bytes=100 * 1024 * 1024),
    )(A_x, A_wqkv, A_wo, B_w1.T, B_b1, B_w2)
```

```python
import jax
import jax.numpy as jnp
from jax.experimental import pallas as pl
from jax.experimental.pallas import tpu as pltpu

S, D, F = 2048, 512, 1376
H, DH, W, DIL = 32, 16, 8, 2
FP = 1408
T = 128
NB = S // T
H2 = T // 2
CH = 16
LNCH = 32
HALO = 16
OSPLIT = 2
LOG2E = 1.4426950408889634
SCHEDULE = """
    S[x0,x1,wq,wk,x2,x3,wv,wo,x4,x5,b1,w1,x6,x7,w2,x8,x9,x10,x11,x12,x13,x14,x15]
    B[x0,x1,wq] Mq Q1 Q0
    B[wk,x2,x3] Pk Q2 Q3 K0 K1 K2
    B[wv,wo,x4,x5] Pv K3 V0 V1 V2 Po K4 V3 V4 V5 K5 WO0 WO1 Q4 WO2 WO3 L2_0 L2_1 Q5 L2_2
    B[b1,w1,x6,x7] Fb W1_0 W1_1 L2_3
    B[w2,x8,x9,x10,x11,x12,x13,x14,x15] W2_0 W1_2 Q6 K6 W2_1 V6 W1_3 V7 W2_2 WO4 Q7 K7 W1_4 W2_3 WO5 V8 Q8 K8 W2_4
    W1_5 WO6 V9 K9 Q9 W2_5 W1_6 WO7 V10 Q10 K10 W2_6 W1_7 WO8 V11 Q11 K11 W2_7 W1_8 WO9 V12 Q12 K12 W2_8 W1_9 WO10
    V13 Q13 K13 W2_9 W1_10 WO11 V14 Q14 K14 W2_10 W1_11 WO12 V15 Q15 K15 W2_11 W1_12 WO13 W2_12 W1_13 WO14 W2_13
    W1_14 WO15 W2_14 W1_15 W2_15
"""
NT = (((1,), (1,)), ((), ()))
bf16, f32, u32 = jnp.bfloat16, jnp.float32, jnp.uint32


def _schedule():
    return SCHEDULE.split()


def _pieces(spec, n):
    v = [int(t) for t in spec.split(":")]
    return (v[0], 0, n) if len(v) == 1 else tuple(v)


def _layernorm(x):
    m = jnp.mean(x, axis=-1, keepdims=True)
    xc = x - m
    v = jnp.mean(xc * xc, axis=-1, keepdims=True)
    return xc * jax.lax.rsqrt(v + 1e-5)


def _mish(h):
    e = jnp.exp2(jnp.minimum(h * LOG2E, 60.0))
    n = e * (e + 2.0)
    return h * (n * pltpu.reciprocal(n + 2.0, approx=True))


def _as_bf16(x):
    return pltpu.bitcast(x, bf16)


def _as_u32(x):
    return pltpu.bitcast(x, u32)


def _kernel(x_hbm, wqkv_hbm, wo_hbm, w1t_hbm, b1_hbm, w2_hbm, o_hbm,
            x_buf, o_buf, wraw, wtmp, woraw, wqkvT, wo_p, w1t, b1v, b1f, w2,
            xn_scr, q_scr, k_scr, v_scr, a_scr, h_scr, hn_scr, act_scr, sems, osem):
    groups = [tok[2:-1].split(",") for tok in _schedule() if tok[:2] == "B["]
    sem_of = {name: sems.at[g] for g, names in enumerate(groups) for name in names}

    def in_copies(name):
        sem = sem_of[name]
        if name[0] == "x":
            i = int(name[1:])
            return [pltpu.make_async_copy(x_hbm.at[0, pl.ds(i * T, T), :], x_buf.at[pl.ds(i * T, T), :], sem)]
        if name in ("wq", "wk", "wv"):
            p = "qkv".index(name[1])
            return [pltpu.make_async_copy(wqkv_hbm.at[:, pl.ds(p * D, D)], wraw.at[p].bitcast(bf16), sem)]
        if name == "wo":
            return [pltpu.make_async_copy(wo_hbm.at[:, pl.ds(j * 128, 128)], woraw.at[j].bitcast(bf16), sem)
                    for j in range(4)]
        if name == "w1":
            return [pltpu.make_async_copy(w1t_hbm, w1t.at[pl.ds(0, F // 2)].bitcast(bf16), sem)]
        if name == "w2":
            return [pltpu.make_async_copy(w2_hbm, w2.at[pl.ds(0, F // 2)].bitcast(bf16), sem)]
        assert name == "b1"
        return [pltpu.make_async_copy(b1_hbm, b1v, sem)]

    def out_copies(i):
        rows = pl.ds(i * T, T)
        if i >= NB - OSPLIT:
            return [pltpu.make_async_copy(o_buf.at[rows, pl.ds(c * 128, 128)], o_hbm.at[0, rows, pl.ds(c * 128, 128)],
                                          osem) for c in range(4)]
        return [pltpu.make_async_copy(o_buf.at[rows, :], o_hbm.at[0, rows, :], osem)]

    def unpack(w):
        lo = pltpu.bitcast(w << 16, f32)
        hi = pltpu.bitcast(w & jnp.uint32(0xFFFF0000), f32)
        return lo.astype(bf16), hi.astype(bf16)

    def prep_w_xlu(p):
        for j in range(4):
            wtmp[p, j] = _as_u32(_as_bf16(wraw[p, pl.ds(j * 64, 64), :]).T)
        for j in range(4):
            for dp in range(DH // 2):
                lo, hi = unpack(wtmp[p, j, pl.ds(dp, H, stride=DH // 2), :])
                wqkvT[pl.ds(p * (D // 2) + (2 * dp) * (H // 2), H // 2), j * 128:(j + 1) * 128] = _as_u32(lo)
                wqkvT[pl.ds(p * (D // 2) + (2 * dp + 1) * (H // 2), H // 2), j * 128:(j + 1) * 128] = _as_u32(hi)

    def prep_w_mxu(p):
        mi = jax.lax.broadcasted_iota(jnp.int32, (128, 128), 0)
        ni = jax.lax.broadcasted_iota(jnp.int32, (128, 128), 1)
        sel = jnp.where(ni == (mi % 8) * DH + mi // 8, 1.0, 0.0).astype(bf16)
        for a in range(2):
            outs = [jax.lax.dot_general(sel, _as_bf16(wraw[p, :, i * 128:(i + 1) * 128]), NT, preferred_element_type=f32)
                    for i in (2 * a, 2 * a + 1)]
            for d in range(DH):
                blk = jnp.concatenate([outs[0][d * 8:(d + 1) * 8], outs[1][d * 8:(d + 1) * 8]], axis=0)
                wqkvT[pl.ds((p * D + d * H + 16 * a) // 2, 8), :] = _as_u32(blk.astype(bf16))

    def prep_wo():
        for j in range(4):
            for dp in range(DH // 2):
                lo, hi = unpack(woraw[j, pl.ds(dp, H, stride=DH // 2), :])
                wo_p[pl.ds((2 * dp) * (H // 2), H // 2), j * 128:(j + 1) * 128] = _as_u32(lo)
                wo_p[pl.ds((2 * dp + 1) * (H // 2), H // 2), j * 128:(j + 1) * 128] = _as_u32(hi)

    def ln1(i):
        for r in range(i * T, (i + 1) * T, LNCH):
            xn_scr[pl.ds(r // 2, LNCH // 2), :] = _as_u32(_layernorm(x_buf[pl.ds(r, LNCH), :].astype(f32)).astype(bf16))

    def proj(i, p):
        dst, off = ((q_scr, 0), (k_scr, HALO), (v_scr, HALO))[p]
        for c in range(4):
            xn = _as_bf16(xn_scr[pl.ds(i * H2, H2), :])
            w = _as_bf16(wqkvT[pl.ds((p * D + c * 128) // 2, 64), :])
            dst[c, pl.ds(off + i * T, T), :] = jax.lax.dot_general(xn, w, NT, preferred_element_type=f32)

    def attention(i):
        for r in range(i * T, (i + 1) * T, CH):
            q = [q_scr[c, pl.ds(r, CH), :] for c in range(4)]
            part = []
            for w in range(W):
                acc = None
                for c in range(4):
                    p = q[c] * k_scr[c, pl.ds(HALO + r - DIL * w, CH), :]
                    acc = p if acc is None else acc + p
                part.append(acc)
            part = [p + pltpu.roll(p, 64, 1) for p in part]
            logits = [p + pltpu.roll(p, 32, 1) for p in part]
            for w in range(W):
                if r < DIL * w:
                    pos = jax.lax.broadcasted_iota(jnp.int32, (CH, 128), 0) + (r - DIL * w)
                    logits[w] = jnp.where(pos >= 0, logits[w], -1e30)
            m = logits[0]
            for w in range(1, W):
                m = jnp.maximum(m, logits[w])
            e = [jnp.exp2((logits[w] - m) * (DH ** -0.5 * LOG2E)) for w in range(W)]
            s = e[0]
            for w in range(1, W):
                s = s + e[w]
            rs = pltpu.reciprocal(s, approx=True)
            for c in range(4):
                acc = None
                for w in range(W):
                    p = e[w] * v_scr[c, pl.ds(HALO + r - DIL * w, CH), :]
                    acc = p if acc is None else acc + p
                a_scr[pl.ds(r // 2, CH // 2), c * 128:(c + 1) * 128] = _as_u32((acc * rs).astype(bf16))

    def out_proj(i):
        for c in range(4):
            a = _as_bf16(a_scr[pl.ds(i * H2, H2), :])
            x = x_buf[pl.ds(i * T, T), c * 128:(c + 1) * 128].astype(f32)
            h_scr[pl.ds(i * T, T), c * 128:(c + 1) * 128] = x + jnp.dot(
                a, _as_bf16(wo_p[:, c * 128:(c + 1) * 128]), preferred_element_type=f32)

    def ln2(i):
        for r in range(i * T, (i + 1) * T, LNCH):
            hn_scr[pl.ds(r // 2, LNCH // 2), :] = _as_u32(_layernorm(h_scr[pl.ds(r, LNCH), :]).astype(bf16))

    def ffn1(i, lo, hi):
        for j in range(lo, hi):
            hn = _as_bf16(hn_scr[pl.ds(i * H2, H2), :])
            hh = jax.lax.dot_general(hn, _as_bf16(w1t[pl.ds(j * 64, 64), :]), NT, preferred_element_type=f32)
            hh = hh + b1f[:, j * 128:(j + 1) * 128]
            act_scr[pl.ds(i * H2, H2), j * 128:(j + 1) * 128] = _as_u32(_mish(hh).astype(bf16))

    def ffn2(i, lo, hi):
        cps = out_copies(i)
        for c in range(lo, hi):
            act = _as_bf16(act_scr[pl.ds(i * H2, H2), :])
            y = jnp.dot(act, _as_bf16(w2[:, c * 128:(c + 1) * 128]), preferred_element_type=f32)
            o_buf[pl.ds(i * T, T), c * 128:(c + 1) * 128] = (h_scr[pl.ds(i * T, T), c * 128:(c + 1) * 128] + y).astype(bf16)
            if len(cps) == 4:
                cps[c].start()
        if len(cps) == 1 and hi == 4:
            cps[0].start()

    done = set()

    def once(name, fn, i):
        if (name, i) not in done:
            done.add((name, i))
            fn(i)

    for tok in _schedule():
        if tok[0] in "SB" and tok[1] == "[":
            for name in tok[2:-1].split(","):
                for cp in in_copies(name):
                    cp.start() if tok[0] == "S" else cp.wait()
            if tok[0] == "S":
                zero = jnp.zeros((HALO, 128), f32)
                for c in range(4):
                    k_scr[c, pl.ds(0, HALO), :] = zero
                    v_scr[c, pl.ds(0, HALO), :] = zero
                zpad = jnp.zeros(((FP - F) // 2, D), u32)
                w1t[pl.ds(F // 2, (FP - F) // 2), :] = zpad
                w2[pl.ds(F // 2, (FP - F) // 2), :] = zpad
                b1f[...] = jnp.zeros((1, FP), f32)
        elif tok == "Fb":
            b1f[:, pl.ds(0, F)] = b1v[...].astype(f32).reshape(1, F)
        elif tok == "Po":
            prep_wo()
        elif tok[0] == "P":
            prep_w_xlu("qkv".index(tok[1]))
        elif tok[0] == "M":
            prep_w_mxu("qkv".index(tok[1]))
        elif tok[0] in "QKV":
            i = int(tok[1:])
            once("ln1", ln1, i)
            proj(i, "QKV".index(tok[0]))
            done.add((tok[0], i))
        elif tok[:2] == "WO":
            i = int(tok[2:])
            assert all((n, j) in done for n in "KV" for j in range(max(i - 1, 0), i + 1)) and ("Q", i) in done
            once("att", attention, i)
            out_proj(i)
            done.add(("WO", i))
        elif tok[:3] == "L2_":
            once("ln2", ln2, int(tok[3:]))
        elif tok[:3] == "W1_":
            i, lo, hi = _pieces(tok[3:], FP // 128)
            assert ("WO", i) in done
            once("ln2", ln2, i)
            ffn1(i, lo, hi)
            if hi == FP // 128:
                done.add(("W1", i))
        else:
            assert tok[:3] == "W2_"
            i, lo, hi = _pieces(tok[3:], 4)
            assert ("W1", i) in done
            ffn2(i, lo, hi)
            if hi == 4:
                done.add(("W2", i))
    assert all(("W2", i) in done for i in range(NB))
    for i in range(NB):
        for cp in out_copies(i):
            cp.wait()


@jax.jit
def pallas_sequential_preLN__sliding_local_dilated__dense_activation_mish__prompt_kernel(
    A_x: jax.Array,
    A_wqkv: jax.Array,
    A_wo: jax.Array,
    B_x: jax.Array,
    B_w1: jax.Array,
    B_b1: jax.Array,
    B_w2: jax.Array,
):
    del B_x
    assert A_x.shape == (1, S, D) and B_w1.shape == (D, F)
    hbm = pl.BlockSpec(memory_space=pltpu.HBM)
    return pl.pallas_call(
        _kernel,
        in_specs=[hbm] * 6,
        out_specs=hbm,
        out_shape=jax.ShapeDtypeStruct((1, S, D), A_x.dtype),
        scratch_shapes=[
            pltpu.VMEM((S, D), bf16),
            pltpu.VMEM((S, D), bf16),
            pltpu.VMEM((3, D // 2, D), u32),
            pltpu.VMEM((3, 4, D // 2, 128), u32),
            pltpu.VMEM((4, D // 2, 128), u32),
            pltpu.VMEM((3 * D // 2, D), u32),
            pltpu.VMEM((D // 2, D), u32),
            pltpu.VMEM((FP // 2, D), u32),
            pltpu.VMEM((F,), bf16),
            pltpu.VMEM((1, FP), f32),
            pltpu.VMEM((FP // 2, D), u32),
            pltpu.VMEM((S // 2, D), u32),
            pltpu.VMEM((4, S, 128), f32),
            pltpu.VMEM((4, S + HALO, 128), f32),
            pltpu.VMEM((4, S + HALO, 128), f32),
            pltpu.VMEM((S // 2, D), u32),
            pltpu.VMEM((S, D), f32),
            pltpu.VMEM((S // 2, D), u32),
            pltpu.VMEM((S // 2, FP), u32),
            pltpu.SemaphoreType.DMA((sum(t[:2] == "B[" for t in _schedule()),)),
            pltpu.SemaphoreType.DMA(()),
        ],
        compiler_params=pltpu.CompilerParams(vmem_limit_bytes=100 * 1024 * 1024),
    )(A_x, A_wqkv, A_wo, B_w1.T, B_b1, B_w2)
```
